```python
import os as _os
_os.environ.setdefault("JAX_PLATFORMS", "cpu")
import jax
import jax.numpy as jnp

def _softmax(x, axis=-1):
    return jax.nn.softmax(x, axis=axis)
def _gelu(x):
    return jax.nn.gelu(x, approximate=True)
def _silu(x):
    return jax.nn.silu(x)
def _sigmoid(x):
    return jax.nn.sigmoid(x)
def _layernorm(x, axis=-1, eps=1e-5):
    m = jnp.mean(x, axis=axis, keepdims=True)
    v = jnp.var(x, axis=axis, keepdims=True)
    return (x - m) / jnp.sqrt(v + eps)
def _scatter_add(tgt, idx, src, axis=0):
    return tgt.at[idx].add(src)
def _segment_sum(src, seg, n):
    return jax.ops.segment_sum(src, seg, n)
class _Rng:
    def __init__(self, key):
        self._k = key
    def _next(self):
        self._k, sub = jax.random.split(self._k)
        return sub
    def normal(self, shape):
        return jax.random.normal(self._next(), shape, dtype=jnp.bfloat16)
    def randint(self, lo, hi, shape):
        return jax.random.randint(self._next(), shape, lo, hi, dtype=jnp.int32)
    def uniform(self, shape, lo=0.0, hi=1.0):
        return jax.random.uniform(self._next(), shape, jnp.bfloat16, lo, hi)
    def permutation(self, n):
        return jax.random.permutation(self._next(), n)


kernel_name = 'gated_mix__gqa_block_cached__dense_activation_squared_relu__decode'

def setup_inputs():
    _rng = _Rng(jax.random.key(int.from_bytes(__import__("os").urandom(4), "little")))
    _w = (lambda a: (lambda t: t.astype(jnp.bfloat16) if jnp.issubdtype(t.dtype, jnp.floating) else t)(jnp.asarray(a)))
    def _A_setup():
        B, Sq, D = 4, 1, 512
        Hq, Hkv, Sk, Dh = 32, 8, 4096, 128
        assert Hq % Hkv == 0, (Hq, Hkv)
        return {
            "x": _w((lambda *s: _rng.normal(s) * 0.05)(B, Sq, D)),
            "k_cache": _w((lambda *s: _rng.normal(s) * 3.2)(B, Hkv, Sk, Dh)),
            "v_cache": _w((lambda *s: _rng.normal(s) * 1.6)(B, Hkv, Sk, Dh)),
            "wq": _w((lambda *s: _rng.normal(s) * 3.2)(D, Hq * Dh) * (D ** -0.5)),
            "wo": _w((lambda *s: _rng.normal(s) * 1.6)(Hq * Dh, D) * ((Hq * Dh) ** -0.5)),
        }
    _A_in = _A_setup()

    def _B_setup():
        B, S, D, F = 4, 1, 512, 1792
        return {
            "x": _w((lambda *s: _rng.normal(s) * 0.05)(B, S, D)),
            "w1": _w((lambda *s: _rng.normal(s) * 0.1)(D, F)),
            "b1": _w((lambda *s: _rng.normal(s) * 0.05)(F)),
            "w2": _w((lambda *s: _rng.normal(s) * 0.05)(F, D)),
            "b2": _w((lambda *s: _rng.normal(s) * 0.05)(D)),
        }
    _B_in = _B_setup()

    return {
        "A_x": _A_in["x"],
        "A_k_cache": _A_in["k_cache"],
        "A_v_cache": _A_in["v_cache"],
        "A_wq": _A_in["wq"],
        "A_wo": _A_in["wo"],
        "B_x": _B_in["x"],
        "B_w1": _B_in["w1"],
        "B_b1": _B_in["b1"],
        "B_w2": _B_in["w2"],
        "B_b2": _B_in["b2"],
        "gate_w": _w((lambda *s: _rng.normal(s) * 0.05)(512) * 16.0),
    }

def reference(A_x, A_k_cache, A_v_cache, A_wq, A_wo, B_x, B_w1, B_b1, B_w2, B_b2, gate_w):
    def _A_ref(x, k_cache, v_cache, wq, wo):
        B, Sq, D = x.shape
        Hq, Dh = 32, 128
        Hkv = k_cache.shape[1]
        rep = Hq // Hkv
        q = (lambda x, *d: x.transpose(*d))((x @ wq).reshape(B, Sq, Hq, Dh), 0, 2, 1, 3)
        k = jnp.repeat(k_cache, rep, axis=1)
        v = jnp.repeat(v_cache, rep, axis=1)
        scores = jnp.einsum("bhqd,bhkd->bhqk", q, k) * (Dh ** -0.5)
        p = _softmax(scores, axis=-1)
        o = jnp.einsum("bhqk,bhkd->bhqd", p, v)
        return (lambda x, *d: x.transpose(*d))(o, 0, 2, 1, 3).reshape(B, Sq, Hq * Dh) @ wo

    def _B_ref(x, w1, b1, w2, b2):
        h = jnp.einsum("bsd,df->bsf", x, w1) + b1
        zero = jnp.zeros_like(h)
        r = jnp.where(h > zero, h, zero)
        h = r * r
        out = jnp.einsum("bsf,fd->bsd", h, w2) + b2
        return out

    x = A_x
    g = _sigmoid((x * gate_w).sum(-1, keepdims=True))
    a = _A_ref(x, A_k_cache, A_v_cache, A_wq, A_wo)
    b = _B_ref(x, B_w1, B_b1, B_w2, B_b2)
    return g * a + (1 - g) * b
```

```python
import jax
import jax.numpy as jnp
from jax import lax
import jax.experimental.pallas as pl
import jax.experimental.pallas.tpu as pltpu


def _kernel(x_ref, k_ref, v_ref, wq_ref, wo_ref, w1_ref, b1_ref, w2_ref, b2_ref,
            gw_ref, o_ref, q_scr, acc_scr, ffn_scr, *, rep, dh, scale):
    h = pl.program_id(0)
    b = pl.program_id(1)
    nh = pl.num_programs(0)
    nb = pl.num_programs(1)
    gqa = rep * dh

    @pl.when(jnp.logical_and(h == 0, b == 0))
    def _():
        acc_scr[...] = jnp.zeros_like(acc_scr)

    @pl.when(b == 0)
    def _():
        q_scr[...] = jnp.dot(x_ref[...], wq_ref[...],
                             preferred_element_type=jnp.float32)

    row8 = lax.broadcasted_iota(jnp.int32, (8, dh), 0)
    qrow = jnp.broadcast_to(q_scr[pl.ds(b, 1), :], (8, gqa))
    q8 = jnp.zeros((8, dh), jnp.float32)
    for r in range(rep):
        q8 = jnp.where(row8 == r, qrow[:, r * dh:(r + 1) * dh], q8)
    q8 = q8.astype(jnp.bfloat16)

    k = k_ref[...]
    s = lax.dot_general(q8, k, (((1,), (1,)), ((), ())),
                        preferred_element_type=jnp.float32)
    s = s * scale
    m = jnp.max(s, axis=1, keepdims=True)
    p = jnp.exp(s - m)
    l = jnp.sum(p, axis=1, keepdims=True)
    o8 = jnp.dot(p.astype(jnp.bfloat16), v_ref[...],
                 preferred_element_type=jnp.float32)
    o8 = o8 / l

    lhs = jnp.concatenate(
        [jnp.where(row8 == r, o8, 0.0) for r in range(rep)], axis=1
    ).astype(jnp.bfloat16)
    part = jnp.dot(lhs, wo_ref[...], preferred_element_type=jnp.float32)
    part = jnp.sum(part, axis=0, keepdims=True)
    acc_scr[pl.ds(b, 1), :] += part

    @pl.when(jnp.logical_and(h == 0, b == 1))
    def _():
        x = x_ref[...]
        hdn = jnp.dot(x, w1_ref[...], preferred_element_type=jnp.float32)
        hdn = hdn + b1_ref[...].astype(jnp.float32)
        r_ = jnp.maximum(hdn, 0.0)
        hdn = (r_ * r_).astype(jnp.bfloat16)
        f = jnp.dot(hdn, w2_ref[...], preferred_element_type=jnp.float32)
        ffn_scr[...] = f + b2_ref[...].astype(jnp.float32)

    @pl.when(jnp.logical_and(h == nh - 1, b == nb - 1))
    def _():
        xf = x_ref[...].astype(jnp.float32)
        gl = jnp.sum(xf * gw_ref[...].astype(jnp.float32), axis=1, keepdims=True)
        g = 1.0 / (1.0 + jnp.exp(-gl))
        a = acc_scr[pl.ds(0, xf.shape[0]), :]
        o_ref[...] = (g * a + (1.0 - g) * ffn_scr[...]).astype(o_ref.dtype)


@jax.jit
def pallas_gated_mix__gqa_block_cached__dense_activation_squared_relu__decode_kernel(
    A_x: jax.Array,
    A_k_cache: jax.Array,
    A_v_cache: jax.Array,
    A_wq: jax.Array,
    A_wo: jax.Array,
    B_x: jax.Array,
    B_w1: jax.Array,
    B_b1: jax.Array,
    B_w2: jax.Array,
    B_b2: jax.Array,
    gate_w: jax.Array,
):
    B, Sq, D = A_x.shape
    _, Hkv, S, Dh = A_k_cache.shape
    HqDh = A_wq.shape[1]
    rep = HqDh // Dh // Hkv
    F = B_w1.shape[1]
    gqa = rep * Dh

    x2 = A_x.reshape(B * Sq, D)
    b1, b2, gw = B_b1, B_b2, gate_w

    kern = lambda *refs: _kernel(*refs, rep=rep, dh=Dh, scale=Dh ** -0.5)

    full = lambda h, b: (0, 0)
    out = pl.pallas_call(
        kern,
        grid=(Hkv, B),
        in_specs=[
            pl.BlockSpec((B, D), full),
            pl.BlockSpec((None, None, S, Dh), lambda h, b: (b, h, 0, 0)),
            pl.BlockSpec((None, None, S, Dh), lambda h, b: (b, h, 0, 0)),
            pl.BlockSpec((D, gqa), lambda h, b: (0, h)),
            pl.BlockSpec((gqa, D), lambda h, b: (h, 0)),
            pl.BlockSpec((D, F), full),
            pl.BlockSpec((F,), lambda h, b: (0,)),
            pl.BlockSpec((F, D), full),
            pl.BlockSpec((D,), lambda h, b: (0,)),
            pl.BlockSpec((D,), lambda h, b: (0,)),
        ],
        out_specs=pl.BlockSpec((B, D), full),
        out_shape=jax.ShapeDtypeStruct((B, D), A_x.dtype),
        scratch_shapes=[
            pltpu.VMEM((B, gqa), jnp.float32),
            pltpu.VMEM((8, D), jnp.float32),
            pltpu.VMEM((B, D), jnp.float32),
        ],
        compiler_params=pltpu.CompilerParams(
            dimension_semantics=("arbitrary", "arbitrary"),
            vmem_limit_bytes=64 * 1024 * 1024,
        ),
    )(x2, A_k_cache, A_v_cache, A_wq, A_wo, B_w1, b1, B_w2, b2, gw)
    return out.reshape(B, Sq, D)
```

```python
import jax
import jax.numpy as jnp
from jax import lax
import jax.experimental.pallas as pl
import jax.experimental.pallas.tpu as pltpu

_CHUNK = 1024


def _kernel(x_hbm, b1_hbm, b2_hbm, gw_hbm,
            k_hbm, v_hbm, wq_hbm, wo_hbm, w1_hbm, w2_hbm,
            o_ref,
            x_ref, b1_ref, b2_ref, gw_ref,
            kbuf, vbuf, wqbuf, wobuf, w1buf, w2buf, q_scr, acc_scr, ffn_scr,
            ksem, vsem, wsem, ssem, *, nb, nh, rep, dh, chunk, nc, scale):
    i = pl.program_id(0)
    nstep = nb * nh
    h = i // nb
    b = i % nb
    gqa = rep * dh

    def kv_copies(step, c):
        bb = step % nb
        hh = step // nb
        ck = pltpu.make_async_copy(
            k_hbm.at[bb, hh, pl.ds(c * chunk, chunk), :], kbuf.at[c], ksem.at[c])
        cv = pltpu.make_async_copy(
            v_hbm.at[bb, hh, pl.ds(c * chunk, chunk), :], vbuf.at[c], vsem.at[c])
        return ck, cv

    def wq_copy(hh):
        slot = hh % 2
        return pltpu.make_async_copy(
            wq_hbm.at[:, pl.ds(hh * gqa, gqa)], wqbuf.at[slot], wsem.at[slot])

    def wo_copy(hh):
        slot = hh % 2
        return pltpu.make_async_copy(
            wo_hbm.at[pl.ds(hh * gqa, gqa), :], wobuf.at[slot], wsem.at[2 + slot])

    def w1_copy():
        return pltpu.make_async_copy(w1_hbm, w1buf, wsem.at[4])

    def w2_copy():
        return pltpu.make_async_copy(w2_hbm, w2buf, wsem.at[5])

    def x_copy():
        return pltpu.make_async_copy(x_hbm, x_ref, ssem.at[0])

    def bias_copies():
        return [pltpu.make_async_copy(src, dst, ssem.at[j]) for j, src, dst in
                [(1, b1_hbm, b1_ref), (2, b2_hbm, b2_ref), (3, gw_hbm, gw_ref)]]

    @pl.when(i == 0)
    def _():
        x_copy().start()
        wq_copy(0).start()
        acc_scr[...] = jnp.zeros_like(acc_scr)
        for c in range(nc - 1):
            ck, cv = kv_copies(0, c)
            ck.start()
            cv.start()
        wo_copy(0).start()
        w1_copy().start()
        w2_copy().start()
        for cp_ in bias_copies():
            cp_.start()
        x_copy().wait()

    @pl.when(b == 0)
    def _():
        wq_copy(h).wait()
        q_scr[...] = jnp.dot(x_ref[...], wqbuf[h % 2],
                             preferred_element_type=jnp.float32)
        wo_copy(h).wait()

        @pl.when(h + 1 < nh)
        def _():
            wq_copy(h + 1).start()
            wo_copy(h + 1).start()

    row8 = lax.broadcasted_iota(jnp.int32, (8, dh), 0)
    qrow = jnp.broadcast_to(q_scr[pl.ds(b, 1), :], (8, gqa))
    q8 = jnp.zeros((8, dh), jnp.float32)
    for r in range(rep):
        q8 = jnp.where(row8 == r, qrow[:, r * dh:(r + 1) * dh], q8)
    q8 = q8.astype(jnp.bfloat16)

    m = jnp.full((8, 1), -jnp.inf, jnp.float32)
    l = jnp.zeros((8, 1), jnp.float32)
    o8 = jnp.zeros((8, dh), jnp.float32)
    for c in range(nc):
        nxt = c + nc - 1
        ip = i + nxt // nc
        cp = nxt % nc

        @pl.when(ip < nstep)
        def _():
            ck, cv = kv_copies(ip, cp)
            ck.start()
            cv.start()

        ck, cv = kv_copies(i, c)
        ck.wait()
        s = lax.dot_general(q8, kbuf[c], (((1,), (1,)), ((), ())),
                            preferred_element_type=jnp.float32)
        s = s * scale
        m_new = jnp.maximum(m, jnp.max(s, axis=1, keepdims=True))
        alpha = jnp.exp(m - m_new)
        p = jnp.exp(s - m_new)
        l = alpha * l + jnp.sum(p, axis=1, keepdims=True)
        cv.wait()
        o8 = alpha * o8 + jnp.dot(p.astype(jnp.bfloat16), vbuf[c],
                                  preferred_element_type=jnp.float32)
        m = m_new
    o8 = o8 / l

    lhs = jnp.concatenate(
        [jnp.where(row8 == r, o8, 0.0) for r in range(rep)], axis=1
    ).astype(jnp.bfloat16)
    part = jnp.dot(lhs, wobuf[h % 2], preferred_element_type=jnp.float32)
    part = jnp.sum(part, axis=0, keepdims=True)
    acc_scr[pl.ds(b, 1), :] += part

    @pl.when(i == 2)
    def _():
        for cp_ in bias_copies():
            cp_.wait()
        w1_copy().wait()
        x = x_ref[...]
        hdn = jnp.dot(x, w1buf[...], preferred_element_type=jnp.float32)
        hdn = hdn + b1_ref[...].astype(jnp.float32)
        r_ = jnp.maximum(hdn, 0.0)
        hdn = (r_ * r_).astype(jnp.bfloat16)
        w2_copy().wait()
        f = jnp.dot(hdn, w2buf[...], preferred_element_type=jnp.float32)
        ffn_scr[...] = f + b2_ref[...].astype(jnp.float32)

    @pl.when(i == nstep - 1)
    def _():
        xf = x_ref[...].astype(jnp.float32)
        gl = jnp.sum(xf * gw_ref[...].astype(jnp.float32), axis=1, keepdims=True)
        g = 1.0 / (1.0 + jnp.exp(-gl))
        a = acc_scr[pl.ds(0, xf.shape[0]), :]
        o_ref[...] = (g * a + (1.0 - g) * ffn_scr[...]).astype(o_ref.dtype)


@jax.jit
def pallas_gated_mix__gqa_block_cached__dense_activation_squared_relu__decode_kernel(
    A_x: jax.Array,
    A_k_cache: jax.Array,
    A_v_cache: jax.Array,
    A_wq: jax.Array,
    A_wo: jax.Array,
    B_x: jax.Array,
    B_w1: jax.Array,
    B_b1: jax.Array,
    B_w2: jax.Array,
    B_b2: jax.Array,
    gate_w: jax.Array,
):
    B, Sq, D = A_x.shape
    _, Hkv, S, Dh = A_k_cache.shape
    HqDh = A_wq.shape[1]
    rep = HqDh // Dh // Hkv
    F = B_w1.shape[1]
    gqa = rep * Dh
    chunk = _CHUNK
    nc = S // chunk

    x2 = A_x.reshape(B * Sq, D)

    kern = lambda *refs: _kernel(*refs, nb=B, nh=Hkv, rep=rep, dh=Dh,
                                 chunk=chunk, nc=nc, scale=Dh ** -0.5)

    any_spec = pl.BlockSpec(memory_space=pl.ANY)
    out = pl.pallas_call(
        kern,
        grid=(Hkv * B,),
        in_specs=[
            any_spec, any_spec, any_spec, any_spec,
            any_spec, any_spec, any_spec, any_spec, any_spec, any_spec,
        ],
        out_specs=pl.BlockSpec((B, D), lambda i: (0, 0)),
        out_shape=jax.ShapeDtypeStruct((B, D), A_x.dtype),
        scratch_shapes=[
            pltpu.VMEM((B, D), A_x.dtype),
            pltpu.VMEM((F,), B_b1.dtype),
            pltpu.VMEM((D,), B_b2.dtype),
            pltpu.VMEM((D,), gate_w.dtype),
            pltpu.VMEM((nc, chunk, Dh), A_k_cache.dtype),
            pltpu.VMEM((nc, chunk, Dh), A_v_cache.dtype),
            pltpu.VMEM((2, D, gqa), A_wq.dtype),
            pltpu.VMEM((2, gqa, D), A_wo.dtype),
            pltpu.VMEM((D, F), B_w1.dtype),
            pltpu.VMEM((F, D), B_w2.dtype),
            pltpu.VMEM((B, gqa), jnp.float32),
            pltpu.VMEM((8, D), jnp.float32),
            pltpu.VMEM((B, D), jnp.float32),
            pltpu.SemaphoreType.DMA((nc,)),
            pltpu.SemaphoreType.DMA((nc,)),
            pltpu.SemaphoreType.DMA((6,)),
            pltpu.SemaphoreType.DMA((4,)),
        ],
        compiler_params=pltpu.CompilerParams(
            dimension_semantics=("arbitrary",),
            vmem_limit_bytes=64 * 1024 * 1024,
        ),
    )(x2, B_b1, B_b2, gate_w, A_k_cache, A_v_cache, A_wq, A_wo, B_w1, B_w2)
    return out.reshape(B, Sq, D)
```
